```python
import os as _os
_os.environ.setdefault("JAX_PLATFORMS", "cpu")
import jax
import jax.numpy as jnp

def _softmax(x, axis=-1):
    return jax.nn.softmax(x, axis=axis)
def _gelu(x):
    return jax.nn.gelu(x, approximate=True)
def _silu(x):
    return jax.nn.silu(x)
def _sigmoid(x):
    return jax.nn.sigmoid(x)
def _layernorm(x, axis=-1, eps=1e-5):
    m = jnp.mean(x, axis=axis, keepdims=True)
    v = jnp.var(x, axis=axis, keepdims=True)
    return (x - m) / jnp.sqrt(v + eps)
def _scatter_add(tgt, idx, src, axis=0):
    return tgt.at[idx].add(src)
def _segment_sum(src, seg, n):
    return jax.ops.segment_sum(src, seg, n)
class _Rng:
    def __init__(self, key):
        self._k = key
    def _next(self):
        self._k, sub = jax.random.split(self._k)
        return sub
    def normal(self, shape):
        return jax.random.normal(self._next(), shape, dtype=jnp.bfloat16)
    def randint(self, lo, hi, shape):
        return jax.random.randint(self._next(), shape, lo, hi, dtype=jnp.int32)
    def uniform(self, shape, lo=0.0, hi=1.0):
        return jax.random.uniform(self._next(), shape, jnp.bfloat16, lo, hi)
    def permutation(self, n):
        return jax.random.permutation(self._next(), n)


kernel_name = 'gated_mix__ssm_conv_h3__ssm_conv_h3__prompt'

def setup_inputs():
    _rng = _Rng(jax.random.key(int.from_bytes(__import__("os").urandom(4), "little")))
    _w = (lambda a: (lambda t: t.astype(jnp.bfloat16) if jnp.issubdtype(t.dtype, jnp.floating) else t)(jnp.asarray(a)))
    def _A_setup():
        B, S, D = 1, 2048, 640
        ks = 4
        return {
            "q": _w((lambda *s: _rng.normal(s) * 0.05)(B, S, D)),
            "k": _w((lambda *s: _rng.normal(s) * 0.05)(B, S, D)),
            "v": _w((lambda *s: _rng.normal(s) * 0.05)(B, S, D)),
            "shift_k": _w((lambda *s: _rng.normal(s) * 0.05)(D, ks) * 0.5),
            "ssm_k": _w((lambda *s: _rng.normal(s) * 0.05)(D, S) * (1.0 / S ** 0.5)),
            "ssm_D": _w((lambda *s: _rng.normal(s) * 0.05)(D)),
        }
    _A_in = _A_setup()

    def _B_setup():
        B, S, D = 1, 2048, 640
        ks = 4
        return {
            "q": _w((lambda *s: _rng.normal(s) * 0.05)(B, S, D)),
            "k": _w((lambda *s: _rng.normal(s) * 0.05)(B, S, D)),
            "v": _w((lambda *s: _rng.normal(s) * 0.05)(B, S, D)),
            "shift_k": _w((lambda *s: _rng.normal(s) * 0.05)(D, ks) * 0.5),
            "ssm_k": _w((lambda *s: _rng.normal(s) * 0.05)(D, S) * (1.0 / S ** 0.5)),
            "ssm_D": _w((lambda *s: _rng.normal(s) * 0.05)(D)),
        }
    _B_in = _B_setup()

    return {
        "A_q": _A_in["q"],
        "A_k": _A_in["k"],
        "A_v": _A_in["v"],
        "A_shift_k": _A_in["shift_k"],
        "A_ssm_k": _A_in["ssm_k"],
        "A_ssm_D": _A_in["ssm_D"],
        "B_q": _B_in["q"],
        "B_k": _B_in["k"],
        "B_v": _B_in["v"],
        "B_shift_k": _B_in["shift_k"],
        "B_ssm_k": _B_in["ssm_k"],
        "B_ssm_D": _B_in["ssm_D"],
        "gate_w": _w((lambda *s: _rng.normal(s) * 0.05)(640) * 16.0),
    }

def reference(A_q, A_k, A_v, A_shift_k, A_ssm_k, A_ssm_D, B_q, B_k, B_v, B_shift_k, B_ssm_k, B_ssm_D, gate_w):
    def _A_ref(q, k, v, shift_k, ssm_k, ssm_D):
        B, S, D = q.shape
        ks = shift_k.shape[-1]
        k_pad = jnp.pad(k, ((0, 0), (ks - 1, 0), (0, 0)))
        k_shift = jnp.zeros_like(k)
        for t in range(ks):
            k_shift = k_shift + k_pad[:, t:t + S, :] * shift_k[:, ks - 1 - t][None, None, :]
        kv = k_shift * v
        L = 2 * S
        kv_pad = jnp.pad(kv, ((0, 0), (0, S), (0, 0)))
        kf_pad = jnp.pad(ssm_k, ((0, 0), (0, S)))
        kv_f = (lambda x, axes=(-2,-1): jnp.fft.rfft2(x.astype(jnp.float32), axes=axes))(kv_pad[:, None, :, :], axes=(1, 2))
        kf_f = (lambda x, axes=(-2,-1): jnp.fft.rfft2(x.astype(jnp.float32), axes=axes))(kf_pad[:, None, :], axes=(1, 2))
        kf_f = (lambda x, *d: x.transpose(*d))(kf_f, 1, 2, 0)
        y_f = kv_f * kf_f[None, :, :, :]
        y = (lambda x, s, axes=(-2,-1): jnp.fft.irfft2(x, s=s, axes=axes).astype(jnp.bfloat16))(y_f, (1, L), axes=(1, 2))[:, 0, :S, :]
        y = y + kv * ssm_D[None, None, :]
        return q * y

    def _B_ref(q, k, v, shift_k, ssm_k, ssm_D):
        B, S, D = q.shape
        ks = shift_k.shape[-1]
        k_pad = jnp.pad(k, ((0, 0), (ks - 1, 0), (0, 0)))
        k_shift = jnp.zeros_like(k)
        for t in range(ks):
            k_shift = k_shift + k_pad[:, t:t + S, :] * shift_k[:, ks - 1 - t][None, None, :]
        kv = k_shift * v
        L = 2 * S
        kv_pad = jnp.pad(kv, ((0, 0), (0, S), (0, 0)))
        kf_pad = jnp.pad(ssm_k, ((0, 0), (0, S)))
        kv_f = (lambda x, axes=(-2,-1): jnp.fft.rfft2(x.astype(jnp.float32), axes=axes))(kv_pad[:, None, :, :], axes=(1, 2))
        kf_f = (lambda x, axes=(-2,-1): jnp.fft.rfft2(x.astype(jnp.float32), axes=axes))(kf_pad[:, None, :], axes=(1, 2))
        kf_f = (lambda x, *d: x.transpose(*d))(kf_f, 1, 2, 0)
        y_f = kv_f * kf_f[None, :, :, :]
        y = (lambda x, s, axes=(-2,-1): jnp.fft.irfft2(x, s=s, axes=axes).astype(jnp.bfloat16))(y_f, (1, L), axes=(1, 2))[:, 0, :S, :]
        y = y + kv * ssm_D[None, None, :]
        return q * y

    x = A_q
    g = _sigmoid((x * gate_w).sum(-1, keepdims=True))
    a = _A_ref(x, A_k, A_v, A_shift_k, A_ssm_k, A_ssm_D)
    b = _B_ref(x, B_k, B_v, B_shift_k, B_ssm_k, B_ssm_D)
    return g * a + (1 - g) * b
```

```python
import functools
import jax
import jax.numpy as jnp
import numpy as np
from jax import lax
from jax.experimental import pallas as pl
from jax.experimental.pallas import tpu as pltpu

S = 2048
D = 640
CT = 128
NT = D // CT
BL = 128
NB = S // BL
NU = 2 * NT
KS = 4
GB = 4
NFT = BL // 8


def _dft_consts():
    f = np.arange(BL)[:, None] + 0.5
    n = np.arange(BL)[None, :]
    ang = 2.0 * np.pi * f * n / (2 * BL)
    C = np.cos(ang).reshape(NFT, 1, 8, BL)
    Sn = -np.sin(ang).reshape(NFT, 1, 8, BL)
    F = np.concatenate([C, Sn], axis=1).reshape(2 * BL, BL)
    G = F.T / BL
    return F.astype(np.float32), G.astype(np.float32)


def _kernel(q_ref, ka_ref, va_ref, ha_ref, kb_ref, vb_ref, hb_ref,
            sk_ref, dd_ref, gw_ref, f_ref, g_ref,
            o_ref,
            xs0, xs1, hs0, hs1, z0, z1, hraw_ref, kbuf_ref, gate_ref, pa_ref, fs_ref, gs_ref):
    s = pl.program_id(0)
    tile_f = jnp.minimum(s // 2, NT - 1)
    tile_i = jnp.clip((s - 2) // 2, 0, NT - 1)
    lane_f = pl.multiple_of(tile_f * CT, CT)
    lane_i = pl.multiple_of(tile_i * CT, CT)
    xs = (xs0, xs1)
    hs = (hs0, hs1)
    zs = (z0, z1)
    kvh = ((ka_ref, va_ref, ha_ref), (kb_ref, vb_ref, hb_ref))

    def gate(t):
        r0 = pl.multiple_of(t * BL, BL)
        ones = jnp.ones((D, CT), jnp.bfloat16)
        gw = gw_ref[...].astype(jnp.float32)
        xb = q_ref[pl.ds(r0, BL), :]
        prod = (xb.astype(jnp.float32) * gw).astype(jnp.bfloat16)
        ssum = jnp.dot(prod, ones, preferred_element_type=jnp.float32)
        ssum = ssum.astype(jnp.bfloat16).astype(jnp.float32)
        gate_ref[pl.ds(r0, BL), :] = jax.nn.sigmoid(ssum).astype(jnp.bfloat16).astype(jnp.float32)

    def elem(t, b):
        k_ref, v_ref, _ = kvh[b]
        skv = sk_ref[b * 8:b * 8 + 8, pl.ds(lane_f, CT)].astype(jnp.float32)
        r0 = pl.multiple_of(t * BL, BL)
        rp = pl.multiple_of(jnp.maximum(t * BL - 16, 0), 16)
        kc = k_ref[pl.ds(r0, BL), :].astype(jnp.float32)
        kp = k_ref[pl.ds(rp, 16), :].astype(jnp.float32)
        kp = jnp.where(t > 0, kp, 0.0)
        vc = v_ref[pl.ds(r0, BL), :].astype(jnp.float32)
        kbuf_ref[0:8, :] = kp[8:16]
        kbuf_ref[8:8 + BL, :] = kc
        acc = kc * skv[0:1]
        for j in range(1, KS):
            acc = acc + kbuf_ref[8 - j:8 - j + BL, :] * skv[j:j + 1]
        return (acc * vc).astype(jnp.bfloat16)

    def fwd(t, b, kv):
        h_ref = kvh[b][2]
        F = fs_ref[...]
        r0 = pl.multiple_of(t * BL, BL)
        xs[b][t] = jnp.dot(F, kv, preferred_element_type=jnp.float32)
        hblk = h_ref[:, pl.ds(r0, BL)]
        hsp = lax.dot_general(F, hblk, (((1,), (1,)), ((), ())), preferred_element_type=jnp.float32)
        hsp = hsp.reshape(NFT, 2, 8, CT)
        sub_odd = (lax.broadcasted_iota(jnp.int32, (NFT, 8, CT), 1) & 1) == 1
        dvec = dd_ref[b * 8:b * 8 + 8, pl.ds(lane_f, CT)].astype(jnp.float32)[0:1]
        hre = hsp[:, 0] + jnp.where(t == 0, dvec, 0.0)[None]
        him = hsp[:, 1]
        prev = hraw_ref[...]
        pre = prev[:, 0]
        pim = prev[:, 1]
        pre = jnp.where(t > 0, jnp.where(sub_odd, -pre, pre), 0.0)
        pim = jnp.where(t > 0, jnp.where(sub_odd, -pim, pim), 0.0)
        hs[b][t, :, 0] = hre - pim
        hs[b][t, :, 1] = him + pre
        hraw_ref[:, 0] = hre
        hraw_ref[:, 1] = him

    def mac(t, b):
        xs_ref, hs_ref, z_ref = xs[b], hs[b], zs[b]
        r = pl.multiple_of(t * 16, 16)
        tok = None
        for A in range(NB // GB):
            acc = [[None] * 3 for _ in range(GB)]
            for Ap in range(A + 1):
                xt = []
                for i in range(GB):
                    ap = Ap * GB + i
                    xr = xs_ref[ap, pl.ds(r, 8), :]
                    xi = xs_ref[ap, pl.ds(r + 8, 8), :]
                    if tok is not None:
                        xr = xr + tok
                        xi = xi + tok
                    xt.append((xr, xi, xr + xi))
                ht = {}
                for d in range(max(0, GB * (A - Ap) - GB + 1), GB * (A - Ap) + GB):
                    c = hs_ref[d, t, 0]
                    dd = hs_ref[d, t, 1]
                    ht[d] = (c, dd - c, c + dd)
                for o in range(GB):
                    a = A * GB + o
                    for i in range(GB):
                        ap = Ap * GB + i
                        if ap > a:
                            continue
                        c, dmc, cpd = ht[a - ap]
                        xr, xi, xs_ = xt[i]
                        ks = (c * xs_, xr * dmc, xi * cpd)
                        for k in range(3):
                            acc[o][k] = ks[k] if acc[o][k] is None else acc[o][k] + ks[k]
                tsum = (acc[0][0] + acc[1][1]) + (acc[2][2] + acc[3][0])
                tok = jnp.minimum(jnp.abs(tsum), 0.0)
            for o in range(GB):
                a = A * GB + o
                k1, k2, k3 = acc[o]
                zz = jnp.concatenate([k1 - k3, k1 + k2], axis=0).astype(jnp.bfloat16)
                z_ref[a, pl.ds(r, 16), :] = zz

    def inv(t, b):
        G = gs_ref[...]
        r0 = pl.multiple_of(t * BL, BL)
        y = jnp.dot(G, zs[b][t], preferred_element_type=jnp.float32)
        qb = q_ref[pl.ds(r0, BL), pl.ds(lane_i, CT)].astype(jnp.float32)
        g = gate_ref[pl.ds(r0, BL), :]
        qy = qb * y
        if b == 0:
            pa_ref[pl.ds(r0, BL), :] = g * qy
        else:
            o_ref[pl.ds(r0, BL), :] = (pa_ref[pl.ds(r0, BL), :] + (1.0 - g) * qy).astype(o_ref.dtype)

    def run(fb, mb, ib, do_gate=False):
        def body(t, kv):
            if ib is not None:
                inv(t, ib)
            if fb is not None:
                fwd(t, fb, kv)
                kv = elem(jnp.minimum(t + 1, NB - 1), fb)
            if mb is not None:
                mac(t, mb)
            if do_gate:
                gate(t)
            return kv
        init = elem(0, fb) if fb is not None else 0
        lax.fori_loop(0, NB, body, init, unroll=2)

    @pl.when(s == 0)
    def _():
        hraw_ref[...] = jnp.zeros_like(hraw_ref)
        fs_ref[...] = f_ref[...]
        gs_ref[...] = g_ref[...]
        run(0, None, None, True)

    @pl.when(s == 1)
    def _():
        run(1, 0, None)

    @pl.when(jnp.logical_and(jnp.logical_and(s >= 2, s < NU), s % 2 == 0))
    def _():
        run(0, 1, 0)

    @pl.when(jnp.logical_and(jnp.logical_and(s >= 2, s < NU), s % 2 == 1))
    def _():
        run(1, 0, 1)

    @pl.when(s == NU)
    def _():
        run(None, 1, 0)

    @pl.when(s == NU + 1)
    def _():
        run(None, None, 1)


@jax.jit
def pallas_gated_mix__ssm_conv_h3__ssm_conv_h3__prompt_kernel(A_q, A_k, A_v, A_shift_k, A_ssm_k, A_ssm_D, B_q, B_k, B_v, B_shift_k, B_ssm_k, B_ssm_D, gate_w):
    F, G = _dft_consts()
    F = jnp.asarray(F, jnp.bfloat16)
    G = jnp.asarray(G, jnp.bfloat16)
    q = A_q.reshape(S, D)
    pad4 = jnp.zeros((4, D), jnp.bfloat16)
    sk = jnp.concatenate([A_shift_k.T, pad4, B_shift_k.T, pad4], axis=0)
    pad7 = jnp.zeros((7, D), jnp.bfloat16)
    dd = jnp.concatenate([A_ssm_D.reshape(1, D), pad7, B_ssm_D.reshape(1, D), pad7], axis=0)
    gw = gate_w.reshape(1, D)

    ia = lambda s: jnp.minimum(s // 2, NT - 1)
    ib = lambda s: jnp.clip((s - 1) // 2, 0, NT - 1)
    io = lambda s: jnp.clip((s - 3) // 2, 0, NT - 1)
    sd = lambda idx: pl.BlockSpec((S, CT), lambda s: (0, idx(s)))
    hd = lambda idx: pl.BlockSpec((CT, S), lambda s: (idx(s), 0))
    full = lambda shp: pl.BlockSpec(shp, lambda s: (0,) * len(shp))
    xspec = pltpu.VMEM((NB, 2 * BL, CT), jnp.float32)
    hspec = pltpu.VMEM((NB, NFT, 2, 8, CT), jnp.float32)
    zspec = pltpu.VMEM((NB, 2 * BL, CT), jnp.bfloat16)
    out = pl.pallas_call(
        _kernel,
        grid=(NU + 2,),
        in_specs=[full((S, D)), sd(ia), sd(ia), hd(ia), sd(ib), sd(ib), hd(ib),
                  full((16, D)), full((16, D)), full((1, D)), full((2 * BL, BL)), full((BL, 2 * BL))],
        out_specs=sd(io),
        out_shape=jax.ShapeDtypeStruct((S, D), jnp.bfloat16),
        scratch_shapes=[
            xspec, xspec, hspec, hspec, zspec, zspec,
            pltpu.VMEM((NFT, 2, 8, CT), jnp.float32),
            pltpu.VMEM((8 + BL, CT), jnp.float32),
            pltpu.VMEM((S, CT), jnp.float32),
            pltpu.VMEM((S, CT), jnp.float32),
            pltpu.VMEM((2 * BL, BL), jnp.bfloat16),
            pltpu.VMEM((BL, 2 * BL), jnp.bfloat16),
        ],
        compiler_params=pltpu.CompilerParams(
            dimension_semantics=("arbitrary",), vmem_limit_bytes=100 * 1024 * 1024),
    )(q, A_k.reshape(S, D), A_v.reshape(S, D), A_ssm_k, B_k.reshape(S, D), B_v.reshape(S, D), B_ssm_k,
      sk, dd, gw, F, G)
    return out.reshape(1, S, D)
```

```python
import jax
import jax.numpy as jnp
import numpy as np
from jax import lax
from jax.experimental import pallas as pl
from jax.experimental.pallas import tpu as pltpu

S = 2048
D = 640
CT = 128
NT = D // CT
BL = 128
NB = S // BL
NU = 2 * NT
KS = 4
GB = 4
NFT = BL // 8


def _dft_consts():
    f = np.arange(BL)[:, None] + 0.5
    n = np.arange(BL)[None, :]
    ang = 2.0 * np.pi * f * n / (2 * BL)
    C = np.cos(ang).reshape(NFT, 1, 8, BL)
    Sn = -np.sin(ang).reshape(NFT, 1, 8, BL)
    F = np.concatenate([C, Sn], axis=1).reshape(2 * BL, BL)
    G = F.T / BL
    return F.astype(np.float32), G.astype(np.float32)


def _kernel(q_hbm, ka_hbm, va_hbm, ha_hbm, kb_hbm, vb_hbm, hb_hbm,
            skt_ref, da_ref, db_ref, gw_ref, f_ref, g_ref,
            o_ref,
            xs0, xs1, hs0, hs1, z0, z1, hraw_ref, kbuf_ref, gate_ref, pa_ref, fs_ref, gs_ref,
            q_ref, ka_ref, va_ref, ha_ref, kb_ref, vb_ref, hb_ref, prm_ref, sems):
    s = pl.program_id(0)

    def copies(b, tile):
        lane = pl.multiple_of(tile * CT, CT)
        k_h, v_h, h_h = ((ka_hbm, va_hbm, ha_hbm), (kb_hbm, vb_hbm, hb_hbm))[b]
        k_v, v_v, h_v = ((ka_ref, va_ref, ha_ref), (kb_ref, vb_ref, hb_ref))[b]
        return (pltpu.make_async_copy(k_h.at[:, pl.ds(lane, CT)], k_v, sems.at[3 * b]),
                pltpu.make_async_copy(v_h.at[:, pl.ds(lane, CT)], v_v, sems.at[3 * b + 1]),
                pltpu.make_async_copy(h_h.at[pl.ds(lane, CT), :], h_v, sems.at[3 * b + 2]))

    def q_copy():
        return pltpu.make_async_copy(q_hbm, q_ref, sems.at[6])

    tile_f = jnp.minimum(s // 2, NT - 1)
    tile_i = jnp.clip((s - 2) // 2, 0, NT - 1)
    lane_f = pl.multiple_of(tile_f * CT, CT)
    lane_i = pl.multiple_of(tile_i * CT, CT)
    xs = (xs0, xs1)
    hs = (hs0, hs1)
    zs = (z0, z1)
    kvh = ((ka_ref, va_ref, ha_ref), (kb_ref, vb_ref, hb_ref))

    def gate(t):
        r0 = pl.multiple_of(t * BL, BL)
        gw = prm_ref[0:8, :][5:6]
        xb = q_ref[pl.ds(r0, BL), :]
        prod = (xb.astype(jnp.float32) * gw).astype(jnp.bfloat16).astype(jnp.float32)
        part = prod[:, 0:CT]
        for j in range(1, NT):
            part = part + prod[:, j * CT:(j + 1) * CT]
        ssum = jnp.sum(part, axis=1, keepdims=True)
        ssum = ssum.astype(jnp.bfloat16).astype(jnp.float32)
        gv = jax.nn.sigmoid(ssum).astype(jnp.bfloat16).astype(jnp.float32)
        gate_ref[pl.ds(r0, BL), :] = jnp.broadcast_to(gv, (BL, CT))

    def elem(t, b):
        k_ref, v_ref, _ = kvh[b]
        skv = prm_ref[b * 8:b * 8 + 8, pl.ds(lane_f, CT)]
        r0 = pl.multiple_of(t * BL, BL)
        rp = pl.multiple_of(jnp.maximum(t * BL - 16, 0), 16)
        kc = k_ref[pl.ds(r0, BL), :].astype(jnp.float32)
        kp = k_ref[pl.ds(rp, 16), :].astype(jnp.float32)
        kp = jnp.where(t > 0, kp, 0.0)
        vc = v_ref[pl.ds(r0, BL), :].astype(jnp.float32)
        kbuf_ref[0:8, :] = kp[8:16]
        kbuf_ref[8:8 + BL, :] = kc
        acc = kc * skv[0:1]
        for j in range(1, KS):
            acc = acc + kbuf_ref[8 - j:8 - j + BL, :] * skv[j:j + 1]
        return (acc * vc).astype(jnp.bfloat16)

    def fwd(t, b, kv):
        h_ref = kvh[b][2]
        F = fs_ref[...]
        r0 = pl.multiple_of(t * BL, BL)
        xs[b][t] = jnp.dot(F, kv, preferred_element_type=jnp.float32)
        hblk = h_ref[:, pl.ds(r0, BL)]
        hsp = lax.dot_general(F, hblk, (((1,), (1,)), ((), ())), preferred_element_type=jnp.float32)
        hsp = hsp.reshape(NFT, 2, 8, CT)
        sub_odd = (lax.broadcasted_iota(jnp.int32, (NFT, 8, CT), 1) & 1) == 1
        dvec = prm_ref[b * 8:b * 8 + 8, pl.ds(lane_f, CT)][4:5]
        hre = hsp[:, 0] + jnp.where(t == 0, dvec, 0.0)[None]
        him = hsp[:, 1]
        prev = hraw_ref[...]
        pre = prev[:, 0]
        pim = prev[:, 1]
        pre = jnp.where(t > 0, jnp.where(sub_odd, -pre, pre), 0.0)
        pim = jnp.where(t > 0, jnp.where(sub_odd, -pim, pim), 0.0)
        hs[b][t, :, 0] = hre - pim
        hs[b][t, :, 1] = him + pre
        hraw_ref[:, 0] = hre
        hraw_ref[:, 1] = him

    def mac(t, b):
        xs_ref, hs_ref, z_ref = xs[b], hs[b], zs[b]
        r = pl.multiple_of(t * 16, 16)
        tok = None
        for A in reversed(range(NB // GB)):
            acc = [[None] * 3 for _ in range(GB)]
            for Ap in range(A + 1):
                xt = []
                for i in range(GB):
                    ap = Ap * GB + i
                    xr = xs_ref[ap, pl.ds(r, 8), :]
                    xi = xs_ref[ap, pl.ds(r + 8, 8), :]
                    if tok is not None:
                        xr = xr + tok
                    xt.append((xr, xi, xr + xi))
                ht = {}
                for d in range(max(0, GB * (A - Ap) - GB + 1), GB * (A - Ap) + GB):
                    c = hs_ref[d, t, 0]
                    dd = hs_ref[d, t, 1]
                    ht[d] = (c, dd - c, c + dd)
                for o in range(GB):
                    a = A * GB + o
                    for i in range(GB):
                        ap = Ap * GB + i
                        if ap > a:
                            continue
                        c, dmc, cpd = ht[a - ap]
                        xr, xi, xs_ = xt[i]
                        ks = (c * xs_, xr * dmc, xi * cpd)
                        for k in range(3):
                            acc[o][k] = ks[k] if acc[o][k] is None else acc[o][k] + ks[k]
                tsum = (acc[0][0] + acc[1][1]) + (acc[2][2] + acc[3][0])
                tok = jnp.minimum(jnp.abs(tsum), 0.0)
            for o in range(GB):
                a = A * GB + o
                k1, k2, k3 = acc[o]
                zz = jnp.concatenate([k1 - k3, k1 + k2], axis=0).astype(jnp.bfloat16)
                z_ref[a, pl.ds(r, 16), :] = zz

    def inv(t, b):
        G = gs_ref[...]
        r0 = pl.multiple_of(t * BL, BL)
        y = jnp.dot(G, zs[b][t], preferred_element_type=jnp.float32)
        qb = q_ref[pl.ds(r0, BL), pl.ds(lane_i, CT)].astype(jnp.float32)
        g = gate_ref[pl.ds(r0, BL), :]
        qy = qb * y
        if b == 0:
            pa_ref[pl.ds(r0, BL), :] = g * qy
        else:
            o_ref[pl.ds(r0, BL), :] = (pa_ref[pl.ds(r0, BL), :] + (1.0 - g) * qy).astype(o_ref.dtype)

    def run(fb, mb, ib, do_gate=False):
        def body(t, kv):
            if ib is not None:
                inv(t, ib)
            if fb is not None:
                fwd(t, fb, kv)
                kv = elem(jnp.minimum(t + 1, NB - 1), fb)
            if mb is not None:
                mac(t, mb)
            if do_gate:
                gate(t)
            return kv
        init = elem(0, fb) if fb is not None else 0
        lax.fori_loop(0, NB, body, init, unroll=2)

    tile_n = jnp.minimum((s + 1) // 2, NT - 1)

    @pl.when(s == 0)
    def _():
        for c in copies(0, 0):
            c.start()
        for c in copies(1, 0):
            c.start()
        q_copy().start()
        hraw_ref[...] = jnp.zeros_like(hraw_ref)
        prm_ref[...] = jnp.zeros_like(prm_ref)
        skt = skt_ref[...].astype(jnp.float32)
        prm_ref[0:4, :] = skt[0:4]
        prm_ref[8:12, :] = skt[4:8]
        prm_ref[4:5, :] = da_ref[...].astype(jnp.float32).reshape(1, D)
        prm_ref[12:13, :] = db_ref[...].astype(jnp.float32).reshape(1, D)
        prm_ref[5:6, :] = gw_ref[...].astype(jnp.float32).reshape(1, D)
        fs_ref[...] = f_ref[...]
        gs_ref[...] = g_ref[...]
        for c in copies(0, 0):
            c.wait()
        run(0, None, None)

    @pl.when(s == 1)
    def _():
        for c in copies(0, tile_n):
            c.start()
        for c in copies(1, 0):
            c.wait()
        q_copy().wait()
        run(1, 0, None, True)

    @pl.when(jnp.logical_and(jnp.logical_and(s >= 2, s < NU), s % 2 == 0))
    def _():
        for c in copies(1, tile_n):
            c.start()
        for c in copies(0, tile_f):
            c.wait()
        run(0, 1, 0)

    @pl.when(jnp.logical_and(jnp.logical_and(s >= 2, s < NU), s % 2 == 1))
    def _():
        @pl.when(s < NU - 1)
        def _():
            for c in copies(0, tile_n):
                c.start()
        for c in copies(1, tile_f):
            c.wait()
        run(1, 0, 1)

    @pl.when(s == NU)
    def _():
        run(None, 1, 0)

    @pl.when(s == NU + 1)
    def _():
        run(None, None, 1)


@jax.jit
def pallas_gated_mix__ssm_conv_h3__ssm_conv_h3__prompt_kernel(A_q, A_k, A_v, A_shift_k, A_ssm_k, A_ssm_D, B_q, B_k, B_v, B_shift_k, B_ssm_k, B_ssm_D, gate_w):
    F, G = _dft_consts()
    F = jnp.asarray(F, jnp.bfloat16)
    G = jnp.asarray(G, jnp.bfloat16)
    q = A_q.reshape(S, D)
    io = lambda s: jnp.clip((s - 3) // 2, 0, NT - 1)
    sd = lambda idx: pl.BlockSpec((S, CT), lambda s: (0, idx(s)))
    anyspec = pl.BlockSpec(memory_space=pl.ANY)
    full = lambda shp: pl.BlockSpec(shp, lambda s: (0,) * len(shp))
    xspec = pltpu.VMEM((NB, 2 * BL, CT), jnp.float32)
    hspec = pltpu.VMEM((NB, NFT, 2, 8, CT), jnp.float32)
    zspec = pltpu.VMEM((NB, 2 * BL, CT), jnp.bfloat16)
    out = pl.pallas_call(
        _kernel,
        grid=(NU + 2,),
        in_specs=[anyspec] * 7 + [
                  full((2 * KS, D)), full((D,)), full((D,)), full((D,)), full((2 * BL, BL)), full((BL, 2 * BL))],
        out_specs=sd(io),
        out_shape=jax.ShapeDtypeStruct((S, D), jnp.bfloat16),
        scratch_shapes=[
            xspec, xspec, hspec, hspec, zspec, zspec,
            pltpu.VMEM((NFT, 2, 8, CT), jnp.float32),
            pltpu.VMEM((8 + BL, CT), jnp.float32),
            pltpu.VMEM((S, CT), jnp.float32),
            pltpu.VMEM((S, CT), jnp.float32),
            pltpu.VMEM((2 * BL, BL), jnp.bfloat16),
            pltpu.VMEM((BL, 2 * BL), jnp.bfloat16),
            pltpu.VMEM((S, D), jnp.bfloat16),
            pltpu.VMEM((S, CT), jnp.bfloat16), pltpu.VMEM((S, CT), jnp.bfloat16), pltpu.VMEM((CT, S), jnp.bfloat16),
            pltpu.VMEM((S, CT), jnp.bfloat16), pltpu.VMEM((S, CT), jnp.bfloat16), pltpu.VMEM((CT, S), jnp.bfloat16),
            pltpu.VMEM((16, D), jnp.float32),
            pltpu.SemaphoreType.DMA((7,)),
        ],
        compiler_params=pltpu.CompilerParams(
            dimension_semantics=("arbitrary",), vmem_limit_bytes=100 * 1024 * 1024),
    )(q, A_k.reshape(S, D), A_v.reshape(S, D), A_ssm_k, B_k.reshape(S, D), B_v.reshape(S, D), B_ssm_k,
      jnp.concatenate([A_shift_k.T, B_shift_k.T], axis=0), A_ssm_D, B_ssm_D, gate_w, F, G)
    return out.reshape(1, S, D)
```
